```python
import os as _os
_os.environ.setdefault("JAX_PLATFORMS", "cpu")
import jax
import jax.numpy as jnp

def _softmax(x, axis=-1):
    return jax.nn.softmax(x, axis=axis)
def _gelu(x):
    return jax.nn.gelu(x, approximate=True)
def _silu(x):
    return jax.nn.silu(x)
def _sigmoid(x):
    return jax.nn.sigmoid(x)
def _layernorm(x, axis=-1, eps=1e-5):
    m = jnp.mean(x, axis=axis, keepdims=True)
    v = jnp.var(x, axis=axis, keepdims=True)
    return (x - m) / jnp.sqrt(v + eps)
def _scatter_add(tgt, idx, src, axis=0):
    return tgt.at[idx].add(src)
def _segment_sum(src, seg, n):
    return jax.ops.segment_sum(src, seg, n)
class _Rng:
    def __init__(self, key):
        self._k = key
    def _next(self):
        self._k, sub = jax.random.split(self._k)
        return sub
    def normal(self, shape):
        return jax.random.normal(self._next(), shape, dtype=jnp.bfloat16)
    def randint(self, lo, hi, shape):
        return jax.random.randint(self._next(), shape, lo, hi, dtype=jnp.int32)
    def uniform(self, shape, lo=0.0, hi=1.0):
        return jax.random.uniform(self._next(), shape, jnp.bfloat16, lo, hi)
    def permutation(self, n):
        return jax.random.permutation(self._next(), n)


kernel_name = 'sequential_preLN__sliding_block__glu_gated_glu__prompt'

def setup_inputs():
    _rng = _Rng(jax.random.key(int.from_bytes(__import__("os").urandom(4), "little")))
    _w = (lambda a: (lambda t: t.astype(jnp.bfloat16) if jnp.issubdtype(t.dtype, jnp.floating) else t)(jnp.asarray(a)))
    def _A_setup():
        B, S, D = 1, 2048, 640
        return {
            "x": _w((lambda *s: _rng.normal(s) * 0.05)(B, S, D)),
            "wqkv": _w((lambda *s: _rng.normal(s) * 0.05)(D, 3 * D)),
            "wo": _w((lambda *s: _rng.normal(s) * 0.05)(D, D)),
        }
    _A_in = _A_setup()

    def _B_setup():
        B, S, D, F = 1, 2048, 640, 1728
        return {
            "x": _w((lambda *s: _rng.normal(s) * 0.05)(B, S, D)),
            "w_gate": _w((lambda *s: _rng.normal(s) * 0.05)(D, F)),
            "w_up": _w((lambda *s: _rng.normal(s) * 0.05)(D, F)),
            "w_down": _w((lambda *s: _rng.normal(s) * 0.05)(F, D)),
        }
    _B_in = _B_setup()

    return {
        "A_x": _A_in["x"],
        "A_wqkv": _A_in["wqkv"],
        "A_wo": _A_in["wo"],
        "B_x": _B_in["x"],
        "B_w_gate": _B_in["w_gate"],
        "B_w_up": _B_in["w_up"],
        "B_w_down": _B_in["w_down"],
    }

def reference(A_x, A_wqkv, A_wo, B_x, B_w_gate, B_w_up, B_w_down):
    def _A_ref(x, wqkv, wo):
        B, S, D = x.shape
        H = 32; Dh = D // H; W = 256
        qkv = (lambda x, *d: x.transpose(*d))((x @ wqkv).reshape(B, S, 3, H, Dh), 2, 0, 3, 1, 4)
        q, k, v = qkv[0], qkv[1], qkv[2]
        scores = jnp.einsum("bhqd,bhkd->bhqk", q, k) * (Dh ** -0.5)
        idx = jnp.arange(S)
        mask = (idx[:, None] - idx[None, :] >= 0) & (idx[:, None] - idx[None, :] < W)
        scores = jnp.where(mask[None, None], scores, -1e9)
        p = _softmax(scores, axis=-1)
        o = jnp.einsum("bhqk,bhkd->bhqd", p, v)
        return (lambda x, *d: x.transpose(*d))(o, 0, 2, 1, 3).reshape(B, S, D) @ wo

    def _B_ref(x, w_gate, w_up, w_down):
        g = jnp.einsum("bsd,df->bsf", x, w_gate)
        u = jnp.einsum("bsd,df->bsf", x, w_up)
        h = _sigmoid(g) * u
        return jnp.einsum("bsf,fd->bsd", h, w_down)

    x = A_x
    h = x + _A_ref(_layernorm(x, axis=-1), A_wqkv, A_wo)
    h2 = h + _B_ref(_layernorm(h, axis=-1), B_w_gate, B_w_up, B_w_down)
    return h2
```

```python
import functools
import jax
import jax.numpy as jnp
from jax import lax
import jax.experimental.pallas as pl
import jax.experimental.pallas.tpu as pltpu

S, D, F = 2048, 640, 1728
H, DH, W = 32, 20, 256
LOG2E = 1.4426950408889634
NEG = -1e30
EPS = 1e-5
f32, bf16, u32 = jnp.float32, jnp.bfloat16, jnp.uint32
NT = (((1,), (1,)), ((), ()))
FM = 1664

def _win_src(i):
    lo = 80 * i
    hi = lo + 80
    g = lo // 128
    if (hi - 1) // 128 == g:
        return (g, g)
    return (g, g + 1)

def _ln(x):
    m = jnp.mean(x, axis=-1, keepdims=True)
    xc = x - m
    v = jnp.mean(xc * xc, axis=-1, keepdims=True)
    return xc * lax.rsqrt(v + EPS)

def _sig(g):
    return 0.5 * jnp.tanh(0.5 * g) + 0.5

def _pk(x):
    return pltpu.bitcast(x.astype(bf16), u32)

def _ipk(a, b, MODE):
    if MODE == 'pe':
        return pltpu.pack_elementwise([a, b], packed_dtype=bf16)
    au = lax.bitcast_convert_type(a, u32)
    bu = lax.bitcast_convert_type(b, u32)
    return (bu & jnp.uint32(0xFFFF0000)) | (au >> 16)

def _pk32(x, MODE):
    if MODE == 'c':
        return _pk(x)
    n = x.shape[0] // 32
    x4 = x.reshape(n, 2, 16, x.shape[1])
    return _ipk(x4[:, 0].reshape(16 * n, x.shape[1]), x4[:, 1].reshape(16 * n, x.shape[1]), MODE)

def _up(x):
    return pltpu.bitcast(x, bf16)

def make_kernel(T, D2, ILV, PACE, MODE, SECOND):
    NQ = T // 128
    NB = S // T
    W2, T2 = W // 2, T // 2
    KR = W2 + T2
    LATE = ('gu', 'wd') if SECOND else ()
    def kernel(x_hbm, wqkv_hbm, wo_hbm, wg_hbm, wu_hbm, wd_hbm, o_ref,
               x_s, wqkv_s, wo_s, wgu_s, wd_s, sems, kbuf, vbuf, qwin, at_ref, attn_s):
        step = pl.program_id(0)

        def xcp(b):
            if isinstance(b, int):
                sl = pl.ds(b * T, T)
            else:
                sl = pl.ds(pl.multiple_of(b * T, T), T)
            return pltpu.make_async_copy(x_hbm.at[sl], x_s.at[sl], sems.at[10 + b])

        def cp(name):
            mk = pltpu.make_async_copy
            if name == 'x0':
                return [xcp(0)]
            if name == 'qk':
                return [mk(wqkv_hbm.at[:, 0:2 * D], wqkv_s.at[:, 0:2 * D], sems.at[1])]
            if name == 'v':
                return [mk(wqkv_hbm.at[:, 2 * D:3 * D], wqkv_s.at[:, 2 * D:3 * D], sems.at[2])]
            if name == 'wo':
                return [mk(wo_hbm, wo_s, sems.at[3])]
            if name == 'x1':
                return [xcp(1)]
            if name == 'gu':
                return [mk(wg_hbm.at[0:FM], wgu_s.at[0:FM], sems.at[5]),
                        mk(wu_hbm.at[0:FM], wgu_s.at[FM:2 * FM], sems.at[6]),
                        mk(wg_hbm.at[FM:F], wgu_s.at[2 * FM:2 * FM + 64], sems.at[7]),
                        mk(wu_hbm.at[FM:F], wgu_s.at[2 * FM + 64:2 * F], sems.at[8])]
            if name == 'wd':
                return [mk(wd_hbm, wd_s, sems.at[9])]
            if name == 'xr':
                return [xcp(b) for b in range(2, NB)]
        def start(*names):
            for n in names:
                for c in cp(n):
                    c.start()
        def wait(*names):
            for n in names:
                for c in cp(n):
                    c.wait()

        def xblk(b):
            if isinstance(b, int):
                return x_s[b * T:(b + 1) * T, :]
            return x_s[pl.ds(pl.multiple_of(b * T, T), T), :]

        def a_ln1(b):
            y = _ln(xblk(b).astype(f32))
            if MODE == 'c':
                return y.astype(bf16), y.astype(bf16)
            yr = y if MODE == 'pe' else y.astype(bf16).astype(f32)
            return y.astype(bf16), _up(_pk32(yr, MODE))

        def a_roll():
            for i in range(8):
                kbuf[i * KR:i * KR + W2, :] = kbuf[i * KR + T2:(i + 1) * KR, :]
            vbuf[:, 0:W] = vbuf[:, T:T + W]

        def a_qk(ln, hook=None):
            lane = lax.broadcasted_iota(jnp.int32, (1, 128), 1)
            qkv = jnp.dot(ln, wqkv_s[:, 0:2 * D], preferred_element_type=f32)
            if hook is not None:
                hook()
            q = qkv[:, 0:D] * (DH ** -0.5 * LOG2E)
            k = qkv[:, D:2 * D]
            for i in range(8):
                gh, gl = _win_src(i)
                kw = k[:, gh * 128:(gh + 1) * 128]
                qw = q[:, gh * 128:(gh + 1) * 128]
                if gl != gh:
                    kw = jnp.where(lane >= 64, kw, k[:, gl * 128:(gl + 1) * 128])
                    qw = jnp.where(lane >= 64, qw, q[:, gl * 128:(gl + 1) * 128])
                kbuf[i * KR + W2:(i + 1) * KR, :] = _pk(kw)
                qwin[i * T2:(i + 1) * T2, :] = _pk(qw)

        def a_v(lnp, hook=None):
            v = jnp.dot(lnp, wqkv_s[:, 2 * D:3 * D], preferred_element_type=f32)
            if hook is not None:
                hook()
            vt = v.T
            row = lax.broadcasted_iota(jnp.int32, (32, 1), 0)
            for h in range(H):
                base = 16 * ((20 * h) // 16)
                off = 20 * h - base
                onerow = 31 if off < 12 else 0
                vb = jnp.where(row == onerow, 1.0, vt[base:base + 32, :])
                vbuf[16 * h:16 * h + 16, W:W + T] = _pk(vb)

        def attn_jobs(first):
            rr = lax.broadcasted_iota(jnp.int32, (32, 128), 0)
            cc = lax.broadcasted_iota(jnp.int32, (32, 128), 1)
            tri = rr > (cc & 31)
            lane = lax.broadcasted_iota(jnp.int32, (16, 128), 1)
            b0 = (lane & 32) == 0
            b1 = (lane & 64) == 0
            zero = jnp.zeros((16, 128), u32)
            never = lax.broadcasted_iota(jnp.int32, (8, 128), 1) < (step >> 8)

            def hmask(h):
                lo = (20 * h) % 128
                hi = lo + 20
                if hi <= 128:
                    return (lane >= lo) & (lane < hi)
                return (lane >= lo) | (lane < hi - 128)

            def rmin(qb, j):
                return max(0, 8 - (qb * 4 + j)) if first else 0

            def qk(i, qb):
                res = []
                for j in range(4):
                    r0 = qb * 64 + 16 * j
                    k0 = i * KR + r0
                    rm = rmin(qb, j)
                    parts = []
                    if rm == 0:
                        parts.append(kbuf[k0:k0 + 16, :])
                    parts.append(kbuf[k0 + 128:k0 + 144, :])
                    lo = max(rm, 1)
                    if lo < 8:
                        parts.append(kbuf[k0 + 16 * lo:k0 + 128, :])
                    lhs = jnp.concatenate(parts, axis=0) if len(parts) > 1 else parts[0]
                    qs = qwin[i * T2 + r0:i * T2 + r0 + 16, :]
                    rhs = jnp.concatenate(
                        [jnp.where(hmask(4 * i + (c - j) % 4), qs, zero) for c in range(4)], axis=0)
                    sp = lax.dot_general(_up(lhs), _up(rhs), NT, preferred_element_type=f32)
                    if rm == 0:
                        sm = jnp.where(tri, sp[0:32], sp[32:64])
                        o = 64
                    else:
                        sm = jnp.where(tri, NEG, sp[0:32])
                        o = 32
                    chunks = [(0, sm)] + [(r, sp[o + 32 * (r - lo):o + 32 * (r - lo + 1)]) for r in range(lo, 8)]
                    run = []
                    cur = None
                    for _, c in chunks:
                        cm = jnp.maximum(jnp.maximum(c[0:8], c[8:16]), jnp.maximum(c[16:24], c[24:32]))
                        cur = cm if cur is None else jnp.maximum(cur, cm)
                        run.append(cur)
                    m8 = jnp.broadcast_to(jnp.max(cur, axis=0, keepdims=True), (8, 128))
                    res.append((chunks, m8, run))
                return res

            def sm_(i, qb, cur, nxt):
                P = [[None] * 9 for _ in range(4)]
                for n in range(8):
                    for j in range(4):
                        chunks, m8, _ = cur[j]
                        if n >= len(chunks):
                            continue
                        r, s = chunks[n]
                        m = m8
                        if PACE and nxt is not None:
                            run = nxt[j][2]
                            m = jnp.where(never, run[min(n, len(run) - 1)], m8)
                        p = jnp.exp2(s.reshape(4, 8, 128) - m[None]).reshape(32, 128)
                        if r > 0:
                            P[j][r] = _pk32(p, MODE)
                        elif rmin(qb, j) == 0:
                            P[j][0] = _pk32(jnp.where(tri, p, 0.0), MODE)
                            P[j][8] = _pk32(jnp.where(tri, 0.0, p), MODE)
                        else:
                            P[j][8] = _pk32(p, MODE)
                return P

            def sel(m, a, b):
                if a is None and b is None:
                    return None
                return jnp.where(m, zero if a is None else a, zero if b is None else b)

            def pv(i, qb, P):
                t0 = (max(0, 2 - qb) if first else 0)
                acc = [None] * 4
                for kt in range(t0, 3):
                    B = [[None] * 4 for _ in range(4)]
                    for r4 in range(4):
                        r = 4 * kt + r4
                        A = [P[j][r - j] if 0 <= r - j <= 8 else None for j in range(4)]
                        C = [sel(b0, A[j], A[(j + 1) % 4]) for j in range(4)]
                        for j in range(4):
                            b = sel(b1, C[j], C[(j + 2) % 4])
                            B[(-j) % 4][r4] = zero if b is None else b
                    for hh in range(4):
                        c0 = qb * 128 + kt * 128
                        h = 4 * i + hh
                        d = jnp.dot(_up(vbuf[16 * h:16 * h + 16, c0:c0 + 128]),
                                    _up(jnp.concatenate(B[hh], axis=0)),
                                    preferred_element_type=f32)
                        acc[hh] = d if acc[hh] is None else acc[hh] + d
                for hh in range(4):
                    off = (20 * hh) % 16
                    onerow = 31 if off < 12 else 0
                    ot = acc[hh]
                    o = ot * pl.reciprocal(ot[onerow:onerow + 1, :], approx=True)
                    if hh:
                        o = pltpu.roll(o, 128 - 32 * hh, 1)
                    at_ref[i, 20 * hh:20 * hh + 20, qb * 128:(qb + 1) * 128] = o[off:off + 20, :]

            units = [(i, qb) for qb in range(NQ) for i in range(8)]
            st = {}
            pt = {}
            jobs = []
            n = len(units)
            for t in range(n + D2):
                def job(t=t):
                    if t < n:
                        st[t] = qk(*units[t])
                    u = t - 1
                    if 0 <= u < n:
                        pt[u] = sm_(*units[u], st.pop(u), st.get(t))
                    u = t - D2
                    if 0 <= u < n:
                        pv(*units[u], pt.pop(u))
                jobs.append(job)
            return jobs

        def a_fin():
            attn_s[...] = _pk(at_ref[...].reshape(D, T).T)

        def f_wo(b):
            h1 = xblk(b).astype(f32) + jnp.dot(_up(attn_s[...]), wo_s[...], preferred_element_type=f32)
            return h1, _ln(h1).astype(bf16)

        def f_gu(ln2):
            gu = lax.dot_general(ln2, wgu_s[...], NT, preferred_element_type=f32)
            hm = _sig(gu[:, 0:FM]) * gu[:, FM:2 * FM]
            ht = _sig(gu[:, 2 * FM:2 * FM + 64]) * gu[:, 2 * FM + 64:2 * F]
            return jnp.concatenate([hm, ht], axis=1).astype(bf16)

        def f_down(h1, hh):
            y = jnp.dot(hh, wd_s[...], preferred_element_type=f32)
            o_ref[...] = (h1 + y).astype(bf16)

        def ffn_jobs(h1, ln2):
            hs = []
            jobs = []
            for c in range(7):
                def job(c=c):
                    if c < 6:
                        w = jnp.concatenate([wgu_s[256 * c:256 * (c + 1), :],
                                             wgu_s[FM + 256 * c:FM + 256 * (c + 1), :]], axis=0)
                        gu = lax.dot_general(ln2, w, NT, preferred_element_type=f32)
                        hs.append(_sig(gu[:, 0:256]) * gu[:, 256:512])
                    else:
                        w = jnp.concatenate([wgu_s[1536:FM, :], wgu_s[FM + 1536:2 * F, :]], axis=0)
                        gu = lax.dot_general(ln2, w, NT, preferred_element_type=f32)
                        hs.append(_sig(gu[:, 0:128]) * gu[:, 128:256])
                        hs.append(_sig(gu[:, 256:320]) * gu[:, 320:384])
                        hs.append(jnp.concatenate(hs[:8], axis=1).astype(bf16))
                jobs.append(job)
            for c in range(5):
                def job(c=c):
                    y = jnp.dot(hs[8], wd_s[:, 128 * c:128 * (c + 1)], preferred_element_type=f32)
                    o_ref[:, 128 * c:128 * (c + 1)] = (h1[:, 128 * c:128 * (c + 1)] + y).astype(bf16)
                jobs.append(job)
            return jobs

        def cwait():
            @pl.when(step == 1)
            def _():
                wait(*LATE)

        def middle(b, second):
            xcp(b).wait()
            h1, ln2 = f_wo(b - 1)
            ln, lnp = a_ln1(b)
            a_roll()
            if SECOND == 3:
                a_v(lnp)
                a_qk(ln, cwait)
            else:
                a_qk(ln)
                a_v(lnp, cwait if SECOND == 1 else None)
            if SECOND == 2:
                cwait()
            if not ILV:
                hh = f_gu(ln2)
                for job in attn_jobs(False):
                    job()
                a_fin()
                f_down(h1, hh)
            else:
                aj = attn_jobs(False)
                fj = ffn_jobs(h1, ln2)
                order = ILV(len(aj), len(fj))
                for kind, idx in order:
                    if kind == 'a':
                        aj[idx]()
                        if idx == len(aj) - 1:
                            a_fin()
                    else:
                        fj[idx]()

        @pl.when(step == 0)
        @jax.named_scope("start")
        def _():
            start('x0', 'qk', 'v', 'wo', 'x1', 'gu', 'wd', 'xr')

        @pl.when(step == 0)
        @jax.named_scope("first")
        def _():
            wait('x0')
            ln, lnp = a_ln1(0)
            wait('qk')
            a_qk(ln)
            wait('v')
            a_v(lnp)
            for job in attn_jobs(True):
                job()
            a_fin()
            wait('wo')
            wait(*[n for n in ('gu', 'wd') if n not in LATE])

        @pl.when(jnp.logical_and(step > 0, step < NB))
        @jax.named_scope("middle")
        def _():
            middle(step, False)

        @pl.when(step == NB)
        @jax.named_scope("last")
        def _():
            h1, ln2 = f_wo(NB - 1)
            hh = f_gu(ln2)
            f_down(h1, hh)
    return kernel

def ilv1(na, nf):
    order = [('f', 0)]
    slots = nf - 1
    k = 0
    for s in range(slots):
        cnt = (na * (s + 1)) // slots - (na * s) // slots
        for _ in range(cnt):
            order.append(('a', k)); k += 1
        order.append(('f', s + 1))
    return order


@jax.jit
def pallas_sequential_preLN__sliding_block__glu_gated_glu__prompt_kernel(
    A_x: jax.Array,
    A_wqkv: jax.Array,
    A_wo: jax.Array,
    B_x: jax.Array,
    B_w_gate: jax.Array,
    B_w_up: jax.Array,
    B_w_down: jax.Array,
):
    T = 256
    NB = S // T
    x = A_x.reshape(S, D)
    hbm = pl.BlockSpec(memory_space=pl.ANY)
    out = pl.pallas_call(
        make_kernel(T, 2, ilv1, 1, 'c', 3),
        grid=(NB + 1,),
        in_specs=[hbm] * 6,
        out_specs=pl.BlockSpec((T, D), lambda i: (jnp.maximum(i - 1, 0), 0)),
        out_shape=jax.ShapeDtypeStruct((S, D), bf16),
        scratch_shapes=[pltpu.VMEM((S, D), bf16),
                        pltpu.VMEM((D, 3 * D), bf16),
                        pltpu.VMEM((D, D), bf16),
                        pltpu.VMEM((2 * F, D), bf16),
                        pltpu.VMEM((F, D), bf16),
                        pltpu.SemaphoreType.DMA((10 + NB,)),
                        pltpu.VMEM((8 * (W + T) // 2, 128), u32),
                        pltpu.VMEM((H * 16, W + T), u32),
                        pltpu.VMEM((8 * T // 2, 128), u32),
                        pltpu.VMEM((8, 80, T), f32),
                        pltpu.VMEM((T // 2, D), u32)],
        compiler_params=pltpu.CompilerParams(dimension_semantics=("arbitrary",),
                                             vmem_limit_bytes=100 * 1024 * 1024),
    )(x, A_wqkv, A_wo, B_w_gate.T, B_w_up.T, B_w_down)
    return out.reshape(1, S, D)
```

```python
import jax
import jax.numpy as jnp
from jax import lax
import jax.experimental.pallas as pl
import jax.experimental.pallas.tpu as pltpu

S, D, F = 2048, 640, 1728
H, DH, W = 32, 20, 256
LOG2E = 1.4426950408889634
NEG = -1e30
EPS = 1e-5
f32, bf16, u32, i32 = jnp.float32, jnp.bfloat16, jnp.uint32, jnp.int32
NT = (((1,), (1,)), ((), ()))
FM = 1664
T = 256
NQ = T // 128
NB = S // T
W2, T2 = W // 2, T // 2
KR = W2 + T2
QC = (0, 512, 1024, 1536, 1920)


def _win_src(i):
    lo = 80 * i
    g = lo // 128
    return (g, g) if (lo + 79) // 128 == g else (g, g + 1)


def _ones_row(h):
    return 31 if (20 * h) % 16 < 12 else 0


def _ln(x):
    m = jnp.mean(x, axis=-1, keepdims=True)
    xc = x - m
    v = jnp.mean(xc * xc, axis=-1, keepdims=True)
    return xc * lax.rsqrt(v + EPS)


def _sig(g):
    return 0.5 * jnp.tanh(0.5 * g) + 0.5


def _pk(x):
    return pltpu.bitcast(x.astype(bf16), u32)


def _up(x):
    return pltpu.bitcast(x, bf16)


def _iota(shape, dim):
    return lax.broadcasted_iota(i32, shape, dim)


def _order_mid(counts, pre="f K Q V"):
    o, t, prev = [pre], 0, []
    for tok, n in zip("g0 g1 g2 g3 g4 g5 g6 d0 d1 d2 d3 D4".split(), counts):
        cur = list(range(t, t + n))
        t += n
        pv = ["p%d" % u for u in prev]
        o += ["k%d" % u for u in cur] + (pv + [tok] if n else [tok] + pv) + ["s%d" % u for u in cur]
        prev = cur
    return " ".join(o)


def _order_first(upto=10, ins=((0, "K"), (6, "Q"), (12, "V"))):
    o, pdone, ins = [], 0, dict(ins)
    for t in range(32):
        if t in ins:
            o.append(ins[t])
        o.append("q%d" % t)
        if t:
            o.append("s%d" % (t - 1))
        while pdone <= t - (3 if t < upto else 2):
            o.append("p%d" % pdone)
            pdone += 1
            if pdone == 16:
                o.append("F")
    return " ".join(o + ["u31", "p30", "p31"])


ORDER_MID = _order_mid([2, 2, 2, 2, 3, 3, 2, 0, 0, 0, 0, 0])
ORDER_FIRST = _order_first()
ORDER_LAST = "f G0 g1 g2 g3 g4 g5 g6 d0 d1 d2 d3 D4"


def make_kernel(order_first, order_mid, order_last, NSS, NSP):
    def kernel(x_hbm, wqkv_hbm, wo_hbm, wg_hbm, wu_hbm, wd_hbm, o_ref,
               x_s, wqkv_s, wo_s, wgu_s, wd_s, sems, kbuf, vbuf, qt, qt0, at_ref, at0_ref,
               attn_s, s_ref, p_ref):
        step = pl.program_id(0)
        zero_rt = step >> 8
        never = _iota((8, 128), 1) < zero_rt

        def rows(b, n):
            if isinstance(b, int):
                return pl.ds(b * n, n)
            return pl.ds(pl.multiple_of(b * n, n), n)

        def stage(ref, r0, val):
            n = val.shape[0]
            pltpu.store(ref.at[pl.ds(r0, n), :], val, mask=_iota((n, 128), 1) >= zero_rt)
            return lambda: ref[r0:r0 + n, :]

        def xcp(b):
            return pltpu.make_async_copy(x_hbm.at[rows(b, T)], x_s.at[rows(b, T)], sems.at[10 + b])

        def cp(name):
            mk = pltpu.make_async_copy
            if name[0] == 'c':
                n = int(name[1])
                return [mk(wqkv_hbm.at[:, QC[n]:QC[n + 1]], wqkv_s.at[:, QC[n]:QC[n + 1]], sems.at[n])]
            if name[0] == 'x':
                return [xcp(int(name[1]))]
            if name == 'wo':
                return [mk(wo_hbm, wo_s, sems.at[4])]
            if name == 'gu':
                return [mk(wg_hbm.at[0:FM], wgu_s.at[0:FM], sems.at[5]),
                        mk(wu_hbm.at[0:FM], wgu_s.at[FM:2 * FM], sems.at[6]),
                        mk(wg_hbm.at[FM:F], wgu_s.at[2 * FM:2 * FM + 64], sems.at[7]),
                        mk(wu_hbm.at[FM:F], wgu_s.at[2 * FM + 64:2 * F], sems.at[8])]
            return [mk(wd_hbm, wd_s, sems.at[9])]

        def wait(*names):
            for n in names:
                for c in cp(n):
                    c.wait()

        def ln1(b):
            return _ln(x_s[rows(b, T), :].astype(f32)).astype(bf16)

        def proj(ln, c0, c1):
            return jnp.dot(ln, wqkv_s[:, c0:c1], preferred_element_type=f32)

        def put_q(q, dst):
            q = q * (DH ** -0.5 * LOG2E)
            hh = (_iota((1, D), 1) * 3277) >> 16
            h0, h1 = (hh & 1) == 1, (hh & 2) == 2
            out = []
            for qb in range(NQ):
                a = [q[qb * 128 + 32 * c:qb * 128 + 32 * c + 32] for c in range(4)]
                b = [jnp.where(h0, a[(c - 1) % 4], a[c]) for c in range(4)]
                out += [jnp.where(h1, b[(c - 2) % 4], b[c]) for c in range(4)]
            dst[...] = _pk(jnp.concatenate(out, axis=0).T)

        def put_k(k, roll, first=False):
            o = 0 if first else W2
            lane = _iota((1, 128), 1)
            for i in range(8):
                gh, gl = _win_src(i)
                w = k[:, gh * 128:(gh + 1) * 128]
                if gl != gh:
                    w = jnp.where(lane >= 64, w, k[:, gl * 128:(gl + 1) * 128])
                if roll:
                    kbuf[i * KR:i * KR + W2, :] = kbuf[i * KR + T2:(i + 1) * KR, :]
                kbuf[i * KR + o:i * KR + o + T2, :] = _pk(w)

        def put_v(v, roll, first=False):
            o = 0 if first else W
            vt = v.T
            row = _iota((32, 1), 0)
            if roll:
                vbuf[:, 0:W] = vbuf[:, T:T + W]
            for h in range(H):
                base = 16 * ((20 * h) // 16)
                vb = jnp.where(row == _ones_row(h), 1.0, vt[base:base + 32, :])
                vbuf[16 * h:16 * h + 16, o:o + T] = _pk(vb)

        class Attn:
            def __init__(self, units):
                self.tri = _iota((32, 128), 0) > (_iota((32, 128), 1) & 31)
                lane = _iota((16, 128), 1)
                self.b0, self.b1 = (lane & 32) == 0, (lane & 64) == 0
                self.zero = jnp.zeros((16, 128), u32)
                self.code = ((_iota((40, 128), 1) >> 5) - ((_iota((40, 128), 0) * 6554) >> 16)) & 3
                self.units, self.st, self.pt = units, {}, {}

            def qk(self, t):
                first, i, qb = self.units[t]
                res, pace = [], []
                for j in range(4):
                    k0 = i * KR + qb * 64 + 16 * j - (W2 if first else 0)
                    rm = max(0, 8 - (qb * 4 + j)) if first else 0
                    lo = max(rm, 1)
                    parts = [kbuf[k0:k0 + 16, :]] if rm == 0 else []
                    parts.append(kbuf[k0 + 128:k0 + 144, :])
                    if lo < 8:
                        parts.append(kbuf[k0 + 16 * lo:k0 + 128, :])
                    lhs = jnp.concatenate(parts, axis=0) if len(parts) > 1 else parts[0]
                    qs = (qt0 if first else qt)[40 * i:40 * i + 40, qb * 128:(qb + 1) * 128]
                    qs = jnp.where(self.code == j, qs, jnp.zeros((40, 128), u32))
                    pos = [self.zero[0:8]] * 8
                    for v in range(5):
                        pos[(5 * i + v) % 8] = qs[8 * v:8 * v + 8]
                    sp = jnp.dot(_up(lhs), _up(jnp.concatenate(pos, axis=0)),
                                 preferred_element_type=f32)
                    o = 64 if rm == 0 else 32
                    edge = jnp.where(self.tri, sp[0:32] if rm == 0 else NEG, sp[o - 32:o])
                    chunks = [(0, edge)] + [(r, sp[o + 32 * (r - lo):o + 32 * (r - lo + 1)])
                                            for r in range(lo, 8)]
                    run = []
                    for _, c in chunks:
                        cm = jnp.maximum(jnp.maximum(c[0:8], c[8:16]), jnp.maximum(c[16:24], c[24:32]))
                        run.append(jnp.maximum(run[-1], cm) if run else cm)
                    m8 = jnp.broadcast_to(jnp.max(run[-1], axis=0, keepdims=True), (8, 128))
                    chunks = [(r, stage(s_ref, ((t % NSS) * 4 + j) * 256 + 32 * r, c)) for r, c in chunks]
                    res.append((chunks, m8, rm))
                    pace.append(run)
                self.st[t] = res
                return pace

            def sm(self, t, pace):
                cur = self.st.pop(t)
                P = [[None] * 9 for _ in range(4)]
                for n in range(8):
                    for j in range(4):
                        chunks, m, rm = cur[j]
                        if n >= len(chunks):
                            continue
                        r, s = chunks[n]
                        if pace is not None:
                            m = jnp.where(never, pace[j][min(n, len(pace[j]) - 1)], m)
                        p = jnp.exp2(s().reshape(4, 8, 128) - m[None]).reshape(32, 128)
                        if r > 0:
                            P[j][r] = _pk(p)
                        elif rm == 0:
                            P[j][0] = _pk(jnp.where(self.tri, p, 0.0))
                            P[j][8] = _pk(jnp.where(self.tri, 0.0, p))
                        else:
                            P[j][8] = _pk(p)
                self.pt[t] = [[None if z is None else stage(p_ref, ((t % NSP) * 4 + j) * 144 + 16 * r, z)
                               for r, z in enumerate(P[j])] for j in range(4)]

            def sel(self, m, a, b):
                if a is None and b is None:
                    return None
                return jnp.where(m, self.zero if a is None else a, self.zero if b is None else b)

            def pv(self, t):
                first, i, qb = self.units[t]
                P = self.pt.pop(t)
                acc = [None] * 4
                for kt in range(max(0, 2 - qb) if first else 0, 3):
                    B = [[None] * 4 for _ in range(4)]
                    for r4 in range(4):
                        r = 4 * kt + r4
                        A = [P[j][r - j] if 0 <= r - j <= 8 else None for j in range(4)]
                        A = [None if a is None else a() for a in A]
                        C = [self.sel(self.b0, A[j], A[(j + 1) % 4]) for j in range(4)]
                        for j in range(4):
                            b = self.sel(self.b1, C[j], C[(j + 2) % 4])
                            B[(-j) % 4][r4] = self.zero if b is None else b
                    c0 = qb * 128 + kt * 128 - (W if first else 0)
                    for hh in range(4):
                        h = 4 * i + hh
                        d = jnp.dot(_up(vbuf[16 * h:16 * h + 16, c0:c0 + 128]),
                                    _up(jnp.concatenate(B[hh], axis=0)),
                                    preferred_element_type=f32)
                        acc[hh] = d if acc[hh] is None else acc[hh] + d
                dst = at0_ref if first else at_ref
                for hh in range(4):
                    off, one = (20 * hh) % 16, _ones_row(hh)
                    o = acc[hh] * (1.0 / acc[hh][one:one + 1, :])
                    if hh:
                        o = pltpu.roll(o, 128 - 32 * hh, 1)
                    dst[i, 20 * hh:20 * hh + 20, qb * 128:(qb + 1) * 128] = o[off:off + 20, :]

        def fin(src, slot):
            attn_s[rows(slot, T2), :] = _pk(src[...].reshape(D, T).T)

        class Ffn:
            def __init__(self, b, split):
                R = T // split
                at = _up(attn_s[rows(b % 2, T2), :])
                x = x_s[rows(b, T), :].astype(f32)
                h1 = [x[s * R:(s + 1) * R] + jnp.dot(at[s * R:(s + 1) * R], wo_s[...],
                                                     preferred_element_type=f32)
                      for s in range(split)]
                self.ln2 = [_ln(h).astype(bf16) for h in h1]
                self.h1 = jnp.concatenate(h1, axis=0) if split > 1 else h1[0]
                self.hs = []

            def gu(self, c, split):
                n = 256 if c < 6 else 128
                w = jnp.concatenate([wgu_s[256 * c:256 * c + n, :],
                                     wgu_s[FM + 256 * c:FM + 256 * c + 256, :]], axis=0)
                ls = self.ln2 if split or len(self.ln2) == 1 else [jnp.concatenate(self.ln2, axis=0)]
                gu = [lax.dot_general(l, w, NT, preferred_element_type=f32) for l in ls]
                gu = jnp.concatenate(gu, axis=0) if len(gu) > 1 else gu[0]
                self.hs.append(_sig(gu[:, 0:n]) * gu[:, n:2 * n])
                if c == 6:
                    self.hs.append(_sig(gu[:, 256:320]) * gu[:, 320:384])
                    self.hh = jnp.concatenate(self.hs, axis=1).astype(bf16)
                cols = [128 * min(j, gu.shape[1] // 128 - 1) for j in range(4)]
                return [[gu[32 * m:32 * m + 8, c0:c0 + 128] for m in range(8)] for c0 in cols]

            def down(self, c, split):
                R = T // split
                for s in range(split):
                    y = jnp.dot(self.hh[s * R:(s + 1) * R], wd_s[:, 128 * c:128 * (c + 1)],
                                preferred_element_type=f32)
                    o_ref[s * R:(s + 1) * R, 128 * c:128 * (c + 1)] = (
                        self.h1[s * R:(s + 1) * R, 128 * c:128 * (c + 1)] + y).astype(bf16)

        def run(order, at, ff, ln, roll):
            pace = None
            for tok in order.split():
                k, n = tok[0], (int(tok[1:]) if tok[1:] else None)
                if k == 'k':
                    at.qk(n)
                elif k == 'q':
                    pace = at.qk(n)
                elif k == 's':
                    at.sm(n, pace)
                elif k == 'u':
                    at.sm(n, None)
                elif k == 'p':
                    at.pv(n)
                elif k in 'gG':
                    pace = ff.gu(n, k == 'G')
                elif k in 'dD':
                    ff.down(n, 2 if k == 'D' else 1)
                elif k == 'f':
                    fin(at_ref, step % 2)
                elif k == 'F':
                    fin(at0_ref, 0)
                elif k == 'Q':
                    put_q(proj(ln, 0, D), qt)
                elif k == 'K':
                    put_k(proj(ln, D, 2 * D), roll)
                elif k == 'V':
                    put_v(proj(ln, 2 * D, 3 * D), roll)

        std = [(False, i, qb) for qb in range(NQ) for i in range(8)]

        @pl.when(step == 0)
        @jax.named_scope("start")
        def _():
            for n in ['x0', 'c0', 'c1', 'c2', 'x1', 'c3', 'wo', 'gu', 'wd'] + ['x%d' % b for b in range(2, NB)]:
                for c in cp(n):
                    c.start()
            s_ref[...] = jnp.zeros(s_ref.shape, f32)
            p_ref[...] = jnp.zeros(p_ref.shape, u32)

        @pl.when(step == 0)
        @jax.named_scope("first")
        def _():
            wait('x0')
            ln = ln1(0)
            zs = []
            for c in range(4):
                wait('c%d' % c)
                if c == 3:
                    wait('x1')
                zs.append(proj(ln, QC[c], QC[c + 1]))
            z = jnp.concatenate(zs, axis=1)
            ln = ln1(1)
            put_k(z[:, D:2 * D], False, True)
            put_q(z[:, 0:D], qt0)
            put_v(z[:, 2 * D:3 * D], False, True)
            units = [(True, i, qb) for qb in range(NQ) for i in range(8)] + std
            run(order_first, Attn(units), None, ln, False)
            wait('wo', 'gu', 'wd')

        @pl.when(jnp.logical_and(step > 0, step < NB - 1))
        @jax.named_scope("middle")
        def _():
            xcp(step + 1).wait()
            ff = Ffn(step - 1, 1)
            run(order_mid, Attn(std), ff, ln1(step + 1), True)

        @pl.when(step >= NB - 1)
        @jax.named_scope("last")
        def _():
            run(order_last, None, Ffn(step - 1, 2), None, None)

    return kernel


@jax.jit
def pallas_sequential_preLN__sliding_block__glu_gated_glu__prompt_kernel(
    A_x: jax.Array,
    A_wqkv: jax.Array,
    A_wo: jax.Array,
    B_x: jax.Array,
    B_w_gate: jax.Array,
    B_w_up: jax.Array,
    B_w_down: jax.Array,
):
    of = ORDER_FIRST
    om = ORDER_MID
    ol = ORDER_LAST
    NSS = 3
    NSP = 4
    hbm = pl.BlockSpec(memory_space=pl.ANY)
    out = pl.pallas_call(
        make_kernel(of, om, ol, NSS, NSP),
        grid=(NB + 1,),
        in_specs=[hbm] * 6,
        out_specs=pl.BlockSpec((T, D), lambda i: (jnp.maximum(i - 1, 0), 0)),
        out_shape=jax.ShapeDtypeStruct((S, D), bf16),
        scratch_shapes=[pltpu.VMEM((S, D), bf16),
                        pltpu.VMEM((D, 3 * D), bf16),
                        pltpu.VMEM((D, D), bf16),
                        pltpu.VMEM((2 * F, D), bf16),
                        pltpu.VMEM((F, D), bf16),
                        pltpu.SemaphoreType.DMA((10 + NB,)),
                        pltpu.VMEM((8 * KR, 128), u32),
                        pltpu.VMEM((H * 16, W + T), u32),
                        pltpu.VMEM((D // 2, T), u32),
                        pltpu.VMEM((D // 2, T), u32),
                        pltpu.VMEM((8, 80, T), f32),
                        pltpu.VMEM((8, 80, T), f32),
                        pltpu.VMEM((2 * T2, D), u32),
                        pltpu.VMEM((NSS * 4 * 256, 128), f32),
                        pltpu.VMEM((NSP * 4 * 144, 128), u32)],
        compiler_params=pltpu.CompilerParams(dimension_semantics=("arbitrary",),
                                             vmem_limit_bytes=100 * 1024 * 1024),
    )(A_x.reshape(S, D), A_wqkv, A_wo, B_w_gate.T, B_w_up.T, B_w_down)
    return out.reshape(1, S, D)
```

```python
import jax
import jax.numpy as jnp
from jax import lax
import jax.experimental.pallas as pl
import jax.experimental.pallas.tpu as pltpu

S, D, F = 2048, 640, 1728
H, DH, W = 32, 20, 256
LOG2E = 1.4426950408889634
NEG = -1e30
EPS = 1e-5
f32, bf16, u32, i32 = jnp.float32, jnp.bfloat16, jnp.uint32, jnp.int32
NT = (((1,), (1,)), ((), ()))
FM = 1664
T = 256
NQ = T // 128
NB = S // T
W2, T2 = W // 2, T // 2
KR = W2 + T2
QC = (0, 512, 1024, 1536, 1920)


def _win_src(i):
    lo = 80 * i
    g = lo // 128
    return (g, g) if (lo + 79) // 128 == g else (g, g + 1)


def _ones_row(h):
    return 23 if h % 2 == 0 else 0


def _ln(x):
    m = jnp.mean(x, axis=-1, keepdims=True)
    xc = x - m
    v = jnp.mean(xc * xc, axis=-1, keepdims=True)
    return xc * lax.rsqrt(v + EPS)


def _sig(g):
    return 0.5 * jnp.tanh(0.5 * g) + 0.5


def _pk(x):
    return pltpu.bitcast(x.astype(bf16), u32)


def _up(x):
    return pltpu.bitcast(x, bf16)


def _iota(shape, dim):
    return lax.broadcasted_iota(i32, shape, dim)


def _order_mid(counts, delay=1, pre="f K Q V"):
    longs, t = [], 0
    for tok, n in zip("g0 g1 g2 g3 g4 g5 g6 d0 d1 d2 d3 D4".split(), counts):
        cur = list(range(t, t + n))
        t += n
        longs += [("k%d" % u, []) for u in cur] + [(tok, cur)]
    o, pend = [pre], []
    for idx, (tok, cur) in enumerate(longs):
        o += [tok] + ["s%d" % u for u in cur]
        pend += [(u, idx + delay) for u in cur]
        if pend and pend[0][1] <= idx and idx + 1 < len(longs) and longs[idx + 1][0][0] != 'g':
            o.append("p%d" % pend.pop(0)[0])
    assert t == 16 and not pend
    return " ".join(o)


def _order_first(upto=10, ins=((0, "K"), (6, "Q"), (12, "V"))):
    o, pdone, ins = [], 0, dict(ins)
    for t in range(32):
        if t in ins:
            o.append(ins[t])
        o.append("q%d" % t)
        if t:
            o.append("s%d" % (t - 1))
        while pdone <= t - (3 if t < upto else 2):
            o.append("p%d" % pdone)
            pdone += 1
            if pdone == 16:
                o.append("F")
    return " ".join(o + ["u31", "p30", "p31"])


def _order_first2(n1, n2, n3, lag=2):
    R = lambda k, a, b: ["%s%d" % (k, u) for u in range(a, b)]
    def Z(a, b):
        o = []
        for n in range(max(len(a), len(b))):
            o += a[n:n + 1] + b[n:n + 1]
        return o
    o = R("k", 0, n1) + ["K"] + R("s", 0, n1)
    o += Z(R("k", n1, n2), R("p", 0, n1)) + ["Q"] + R("s", n1, n2)
    o += Z(R("k", n2, n3), R("p", n1, n2)) + ["V"] + R("s", n2, n3)
    pdone = n2
    for t in range(n3, 32):
        o.append("q%d" % t)
        if t > n3:
            o.append("s%d" % (t - 1))
        cnt = 0
        while pdone <= t - lag and cnt < (2 if pdone < 16 else 1):
            o.append("p%d" % pdone)
            pdone += 1
            cnt += 1
            if pdone == 16:
                o.append("F")
    o.append("u31")
    o += R("p", pdone, 32)
    return " ".join(o)


ORDER_MID = _order_mid([3, 3, 2, 2, 2, 2, 2, 0, 0, 0, 0, 0], 2)
ORDER_FIRST = _order_first2(8, 11, 14)
ORDER_LAST = "f G0 g1 g2 g3 g4 g5 g6 d0 d1 d2 d3 D4"


def make_kernel(order_first, order_mid, order_last, CF, CM, PM, PM6, PMQ):
    def kernel(x_hbm, wqkv_hbm, wo_hbm, wg_hbm, wu_hbm, wd_hbm, o_hbm,
               x_s, wqkv_s, wo_s, wgu_s, wd_s, sems, kbuf, vbuf, qt, qt0, at_ref, at0_ref,
               attn_s, s_ref, p_ref, o_s, osems):
        step = pl.program_id(0)
        zero_rt = step >> 8
        never = _iota((8, 128), 1) < zero_rt

        def rows(b, n):
            if isinstance(b, int):
                return pl.ds(b * n, n)
            return pl.ds(pl.multiple_of(b * n, n), n)

        class Ring:
            def __init__(self, ref, n, cap):
                assert cap * n <= ref.shape[0]
                self.ref, self.n, self.cap, self.ptr, self.live = ref, n, cap, 0, set()

            def put(self, val):
                k, n = self.ptr, self.n
                self.ptr = (k + 1) % self.cap
                assert k not in self.live
                self.live.add(k)
                pltpu.store(self.ref.at[pl.ds(k * n, n), :], val, mask=_iota((n, 128), 1) >= zero_rt)
                return k

            def get(self, k):
                self.live.remove(k)
                return self.ref[k * self.n:(k + 1) * self.n, :]

        def xcp(b):
            return pltpu.make_async_copy(x_hbm.at[rows(b, T)], x_s.at[rows(b, T)], sems.at[10 + b])

        def ocp(b, c):
            return pltpu.make_async_copy(o_s.at[rows(b % 2, T), 128 * c:128 * (c + 1)],
                                         o_hbm.at[rows(b, T), 128 * c:128 * (c + 1)],
                                         osems.at[(b % 2) * 5 + c])

        def ocp_full(b):
            return pltpu.make_async_copy(o_s.at[rows(b % 2, T)], o_hbm.at[rows(b, T)], osems.at[10 + b % 2])

        def cp(name):
            mk = pltpu.make_async_copy
            if name[0] == 'c':
                n = int(name[1])
                return [mk(wqkv_hbm.at[:, QC[n]:QC[n + 1]], wqkv_s.at[:, QC[n]:QC[n + 1]], sems.at[n])]
            if name[0] == 'x':
                return [xcp(int(name[1]))]
            if name == 'wo':
                return [mk(wo_hbm, wo_s, sems.at[4])]
            if name == 'gu':
                return [mk(wg_hbm.at[0:FM], wgu_s.at[0:FM], sems.at[5]),
                        mk(wu_hbm.at[0:FM], wgu_s.at[FM:2 * FM], sems.at[6]),
                        mk(wg_hbm.at[FM:F], wgu_s.at[2 * FM:2 * FM + 64], sems.at[7]),
                        mk(wu_hbm.at[FM:F], wgu_s.at[2 * FM + 64:2 * F], sems.at[8])]
            return [mk(wd_hbm, wd_s, sems.at[9])]

        def wait(*names):
            for n in names:
                for c in cp(n):
                    c.wait()

        def ln1(b):
            return _ln(x_s[rows(b, T), :].astype(f32)).astype(bf16)

        def proj(ln, c0, c1):
            return jnp.dot(ln, wqkv_s[:, c0:c1], preferred_element_type=f32)

        def put_q(q, dst):
            q = q * (DH ** -0.5 * LOG2E)
            hh = (_iota((1, D), 1) * 3277) >> 16
            h0, h1 = (hh & 1) == 1, (hh & 2) == 2
            out = []
            for qb in range(NQ):
                a = [q[qb * 128 + 32 * c:qb * 128 + 32 * c + 32] for c in range(4)]
                b = [jnp.where(h0, a[(c - 1) % 4], a[c]) for c in range(4)]
                out += [jnp.where(h1, b[(c - 2) % 4], b[c]) for c in range(4)]
            dst[...] = _pk(jnp.concatenate(out, axis=0).T)

        def put_k(k, roll, first=False):
            o = 0 if first else W2
            lane = _iota((1, 128), 1)
            for i in range(8):
                gh, gl = _win_src(i)
                w = k[:, gh * 128:(gh + 1) * 128]
                if gl != gh:
                    w = jnp.where(lane >= 64, w, k[:, gl * 128:(gl + 1) * 128])
                if roll:
                    kbuf[i * KR:i * KR + W2, :] = kbuf[i * KR + T2:(i + 1) * KR, :]
                kbuf[i * KR + o:i * KR + o + T2, :] = _pk(w)

        def put_v(v, roll, first=False):
            o = 0 if first else W
            vt = v.T
            row = _iota((24, 1), 0)
            if roll:
                vbuf[:, 0:W] = vbuf[:, T:T + W]
            for h in range(H):
                base = 8 * ((20 * h) // 8)
                vbuf[24 * h:24 * h + 24, o:o + T] = jnp.where(row == _ones_row(h), 1.0, vt[base:base + 24, :])

        class Attn:
            def __init__(self, units, caps):
                self.tri = _iota((32, 128), 0) > (_iota((32, 128), 1) & 31)
                lane = _iota((16, 128), 1)
                self.b0, self.b1 = (lane & 32) == 0, (lane & 64) == 0
                self.zero = jnp.zeros((16, 128), u32)
                self.code = ((_iota((40, 128), 1) >> 5) - ((_iota((40, 128), 0) * 6554) >> 16)) & 3
                self.units, self.st, self.pt = units, {}, {}
                self.sr, self.pr = Ring(s_ref, 32, caps[0]), Ring(p_ref, 16, caps[1])

            def qk(self, t):
                first, i, qb = self.units[t]
                res, pace = [], []
                for j in range(4):
                    k0 = i * KR + qb * 64 + 16 * j - (W2 if first else 0)
                    rm = max(0, 8 - (qb * 4 + j)) if first else 0
                    lo = max(rm, 1)
                    parts = [kbuf[k0:k0 + 16, :]] if rm == 0 else []
                    parts.append(kbuf[k0 + 128:k0 + 144, :])
                    if lo < 8:
                        parts.append(kbuf[k0 + 16 * lo:k0 + 128, :])
                    lhs = jnp.concatenate(parts, axis=0) if len(parts) > 1 else parts[0]
                    qs = (qt0 if first else qt)[40 * i:40 * i + 40, qb * 128:(qb + 1) * 128]
                    qs = jnp.where(self.code == j, qs, jnp.zeros((40, 128), u32))
                    pos = [self.zero[0:8]] * 8
                    for v in range(5):
                        pos[(5 * i + v) % 8] = qs[8 * v:8 * v + 8]
                    sp = jnp.dot(_up(lhs), _up(jnp.concatenate(pos, axis=0)),
                                 preferred_element_type=f32)
                    o = 64 if rm == 0 else 32
                    edge = jnp.where(self.tri, sp[0:32] if rm == 0 else NEG, sp[o - 32:o])
                    chunks = [(0, edge)] + [(r, sp[o + 32 * (r - lo):o + 32 * (r - lo + 1)])
                                            for r in range(lo, 8)]
                    run = []
                    for _, c in chunks:
                        cm = jnp.maximum(jnp.maximum(c[0:8], c[8:16]), jnp.maximum(c[16:24], c[24:32]))
                        run.append(jnp.maximum(run[-1], cm) if run else cm)
                    m8 = jnp.broadcast_to(jnp.max(run[-1], axis=0, keepdims=True), (8, 128))
                    chunks = [(r, self.sr.put(c)) for r, c in chunks]
                    res.append((chunks, m8, rm))
                    pace.append(run)
                self.st[t] = res
                return pace

            def sm(self, t, pace):
                cur = self.st.pop(t)
                P = [[None] * 9 for _ in range(4)]
                for n in range(8):
                    for j in range(4):
                        chunks, m, rm = cur[j]
                        if n >= len(chunks):
                            continue
                        r, s = chunks[n]
                        if pace is not None:
                            m = jnp.where(never, pace[j][min(n, len(pace[j]) - 1)], m)
                        p = jnp.exp2(self.sr.get(s).reshape(4, 8, 128) - m[None]).reshape(32, 128)
                        if r > 0:
                            P[j][r] = _pk(p)
                        elif rm == 0:
                            P[j][0] = _pk(jnp.where(self.tri, p, 0.0))
                            P[j][8] = _pk(jnp.where(self.tri, 0.0, p))
                        else:
                            P[j][8] = _pk(p)
                self.pt[t] = [[None if z is None else self.pr.put(z) for z in P[j]] for j in range(4)]

            def sel(self, m, a, b):
                if a is None and b is None:
                    return None
                return jnp.where(m, self.zero if a is None else a, self.zero if b is None else b)

            def pv(self, t):
                first, i, qb = self.units[t]
                P = self.pt.pop(t)
                acc = [None] * 4
                for kt in range(max(0, 2 - qb) if first else 0, 3):
                    B = [[None] * 4 for _ in range(4)]
                    for r4 in range(4):
                        r = 4 * kt + r4
                        A = [P[j][r - j] if 0 <= r - j <= 8 else None for j in range(4)]
                        A = [None if a is None else self.pr.get(a) for a in A]
                        C = [self.sel(self.b0, A[j], A[(j + 1) % 4]) for j in range(4)]
                        for j in range(4):
                            b = self.sel(self.b1, C[j], C[(j + 2) % 4])
                            B[(-j) % 4][r4] = self.zero if b is None else b
                    c0 = qb * 128 + kt * 128 - (W if first else 0)
                    for hh in range(4):
                        h = 4 * i + hh
                        d = jnp.dot(vbuf[24 * h:24 * h + 24, c0:c0 + 128],
                                    _up(jnp.concatenate(B[hh], axis=0)),
                                    preferred_element_type=f32)
                        acc[hh] = d if acc[hh] is None else acc[hh] + d
                dst = at0_ref if first else at_ref
                for hh in range(4):
                    off, one = (20 * hh) % 8, _ones_row(hh)
                    o = acc[hh] * (1.0 / acc[hh][one:one + 1, :])
                    if hh:
                        o = pltpu.roll(o, 128 - 32 * hh, 1)
                    dst[i, 20 * hh:20 * hh + 20, qb * 128:(qb + 1) * 128] = o[off:off + 20, :]

        def fin(src, slot):
            attn_s[rows(slot, T2), :] = _pk(src[...].reshape(D, T).T)

        class Ffn:
            def __init__(self, b, split):
                R = T // split
                at = _up(attn_s[rows(b % 2, T2), :])
                x = x_s[rows(b, T), :].astype(f32)
                h1 = [x[s * R:(s + 1) * R] + jnp.dot(at[s * R:(s + 1) * R], wo_s[...],
                                                     preferred_element_type=f32)
                      for s in range(split)]
                self.ln2 = [_ln(h).astype(bf16) for h in h1]
                self.h1 = jnp.concatenate(h1, axis=0) if split > 1 else h1[0]
                self.hs = []
                self.b, self.chunked = b, split > 1

            def gu(self, c, split):
                n = 256 if c < 6 else 128
                w = jnp.concatenate([wgu_s[256 * c:256 * c + n, :],
                                     wgu_s[FM + 256 * c:FM + 256 * c + 256, :]], axis=0)
                ls = self.ln2 if split or len(self.ln2) == 1 else [jnp.concatenate(self.ln2, axis=0)]
                gu = [lax.dot_general(l, w, NT, preferred_element_type=f32) for l in ls]
                gu = jnp.concatenate(gu, axis=0) if len(gu) > 1 else gu[0]
                self.hs.append(_sig(gu[:, 0:n]) * gu[:, n:2 * n])
                if c == 6:
                    self.hs.append(_sig(gu[:, 256:320]) * gu[:, 320:384])
                    self.hh = jnp.concatenate(self.hs, axis=1).astype(bf16)
                cols = [128 * min(j, gu.shape[1] // 128 - 1) for j in (PM if c < 6 else PM6)]
                return [[gu[32 * m:32 * m + 8, c0:c0 + 128] for m in range(8)] for c0 in cols]

            def down(self, c, split):
                R = T // split
                for s in range(split):
                    y = jnp.dot(self.hh[s * R:(s + 1) * R], wd_s[:, 128 * c:128 * (c + 1)],
                                preferred_element_type=f32)
                    o_s[rows((self.b % 2) * split + s, R), 128 * c:128 * (c + 1)] = (
                        self.h1[s * R:(s + 1) * R, 128 * c:128 * (c + 1)] + y).astype(bf16)
                if self.chunked:
                    ocp(self.b, c).start()

        def run(order, at, ff, ln, roll):
            pace = None
            for tok in order.split():
                k, n = tok[0], (int(tok[1:]) if tok[1:] else None)
                if k == 'k':
                    at.qk(n)
                elif k == 'q':
                    pace = at.qk(n)
                elif k == 's':
                    at.sm(n, pace)
                elif k == 'u':
                    at.sm(n, None)
                elif k == 'p':
                    at.pv(n)
                elif k in 'gG':
                    pace = ff.gu(n, k == 'G')
                elif k in 'dD':
                    ff.down(n, 2 if k == 'D' else 1)
                elif k == 'f':
                    fin(at_ref, step % 2)
                elif k == 'F':
                    fin(at0_ref, 0)
                elif k in 'QKV':
                    c0 = 'QKV'.index(k) * D
                    z = proj(ln, c0, c0 + D)
                    pace = [[z[32 * m:32 * m + 8, 128 * c:128 * c + 128] for m in range(8)] for c in PMQ]
                    if k == 'Q':
                        put_q(z, qt)
                    elif k == 'K':
                        put_k(z, roll)
                    else:
                        put_v(z, roll)

        std = [(False, i, qb) for qb in range(NQ) for i in range(8)]

        @pl.when(step >= 3)
        def _():
            ocp_full(step - 3).wait()

        @pl.when(step == 0)
        @jax.named_scope("start")
        def _():
            for n in ['x0', 'c0', 'c1', 'c2', 'x1', 'c3', 'wo', 'gu', 'wd'] + ['x%d' % b for b in range(2, NB)]:
                for c in cp(n):
                    c.start()
            s_ref[...] = jnp.zeros(s_ref.shape, f32)
            p_ref[...] = jnp.zeros(p_ref.shape, u32)

        @pl.when(step == 0)
        @jax.named_scope("first")
        def _():
            if order_first is None:
                return
            wait('x0')
            ln = ln1(0)
            zs = []
            for c in range(4):
                wait('c%d' % c)
                if c == 3:
                    wait('x1')
                zs.append(proj(ln, QC[c], QC[c + 1]))
            z = jnp.concatenate(zs, axis=1)
            ln = ln1(1)
            put_k(z[:, D:2 * D], False, True)
            put_q(z[:, 0:D], qt0)
            put_v(z[:, 2 * D:3 * D], False, True)
            units = [(True, i, qb) for qb in range(NQ) for i in range(8)] + std
            run(order_first, Attn(units, CF), None, ln, False)
            wait('wo', 'gu', 'wd')

        @pl.when(jnp.logical_and(step > 0, step < NB - 1))
        @jax.named_scope("middle")
        def _():
            if order_mid is None:
                return
            xcp(step + 1).wait()
            ff = Ffn(step - 1, 1)
            run(order_mid, Attn(std, CM), ff, ln1(step + 1), True)
            ocp_full(step - 1).start()

        @pl.when(step >= NB - 1)
        @jax.named_scope("last")
        def _():
            if order_last is None:
                return
            run(order_last, None, Ffn(step - 1, 2), None, None)

        @pl.when(step == NB)
        def _():
            for b in (NB - 2, NB - 1):
                for c in range(5):
                    ocp(b, c).wait()

    return kernel


@jax.jit
def pallas_sequential_preLN__sliding_block__glu_gated_glu__prompt_kernel(
    A_x: jax.Array,
    A_wqkv: jax.Array,
    A_wo: jax.Array,
    B_x: jax.Array,
    B_w_gate: jax.Array,
    B_w_up: jax.Array,
    B_w_down: jax.Array,
):
    of = ORDER_FIRST
    om = ORDER_MID
    ol = ORDER_LAST
    CF = (96, 180)
    CM = (104, 180)
    PM = (0, 1, 1, 2)
    PM6 = (0, 0, 1, 1)
    NOBC = False
    PMQ = (0, 1, 2, 3)
    hbm = pl.BlockSpec(memory_space=pl.ANY)
    out = pl.pallas_call(
        make_kernel(of, om, ol, CF, CM, PM, PM6, PMQ),
        grid=(NB + 1,),
        in_specs=[hbm] * 6,
        out_specs=hbm,
        out_shape=jax.ShapeDtypeStruct((S, D), bf16),
        scratch_shapes=[pltpu.VMEM((S, D), bf16),
                        pltpu.VMEM((D, 3 * D), bf16),
                        pltpu.VMEM((D, D), bf16),
                        pltpu.VMEM((2 * F, D), bf16),
                        pltpu.VMEM((F, D), bf16),
                        pltpu.SemaphoreType.DMA((10 + NB,)),
                        pltpu.VMEM((8 * KR, 128), u32),
                        pltpu.VMEM((H * 24, W + T), f32),
                        pltpu.VMEM((D // 2, T), u32),
                        pltpu.VMEM((D // 2, T), u32),
                        pltpu.VMEM((8, 80, T), f32),
                        pltpu.VMEM((8, 80, T), f32),
                        pltpu.VMEM((2 * T2, D), u32),
                        pltpu.VMEM((max(CF[0], CM[0]) * 32, 128), f32),
                        pltpu.VMEM((max(CF[1], CM[1]) * 16, 128), u32),
                        pltpu.VMEM((2 * T, D), bf16),
                        pltpu.SemaphoreType.DMA((12,))],
        compiler_params=pltpu.CompilerParams(dimension_semantics=("arbitrary",),
                                             vmem_limit_bytes=100 * 1024 * 1024,
                                             disable_bounds_checks=NOBC),
    )(A_x.reshape(S, D), A_wqkv, A_wo, B_w_gate.T, B_w_up.T, B_w_down)
    return out.reshape(1, S, D)
```

```python
import jax
import jax.numpy as jnp
from jax import lax
import jax.experimental.pallas as pl
import jax.experimental.pallas.tpu as pltpu

S, D, F = 2048, 640, 1728
H, DH, W = 32, 20, 256
LOG2E = 1.4426950408889634
NEG = -1e30
EPS = 1e-5
f32, bf16, u32, i32 = jnp.float32, jnp.bfloat16, jnp.uint32, jnp.int32
NT = (((1,), (1,)), ((), ()))
FM = 1664
T = 256
NQ = T // 128
NB = S // T
W2, T2 = W // 2, T // 2
KR = W2 + T2
QC = (0, 512, 1024, 1536, 1920)


def _win_src(i):
    lo = 80 * i
    g = lo // 128
    return (g, g) if (lo + 79) // 128 == g else (g, g + 1)


def _ones_row(h):
    return 23 if h % 2 == 0 else 0


def _ln(x, scale=None):
    m = jnp.mean(x, axis=-1, keepdims=True)
    xc = x - m
    v = jnp.mean(xc * xc, axis=-1, keepdims=True)
    r = lax.rsqrt(v + EPS)
    return xc * (r if scale is None else r * scale)


def _glu(gh, uh):
    return (jnp.tanh(gh) + 1.0) * uh


def _pk(x):
    return pltpu.bitcast(x.astype(bf16), u32)


def _up(x):
    return pltpu.bitcast(x, bf16)


def _iota(shape, dim):
    return lax.broadcasted_iota(i32, shape, dim)


def _seq(k, a, b):
    return ["%s%d" % (k, u) for u in range(a, b)]


def _zip(a, b):
    return [t for n in range(max(len(a), len(b))) for t in a[n:n + 1] + b[n:n + 1]]


def _order_mid(counts, delay):
    longs, t = [], 0
    for tok, n in zip("g0 g1 g2 g3 g4 g5 g6 d0 d1 d2 d3 D4".split(), counts + [0] * 5):
        longs += [(k, []) for k in _seq("k", t, t + n)] + [(tok, list(range(t, t + n)))]
        t += n
    o, pend = ["f", "K", "Q", "V"], []
    for idx, (tok, cur) in enumerate(longs):
        o += [tok] + ["s%d" % u for u in cur]
        pend += [(u, idx + delay) for u in cur]
        if pend and pend[0][1] <= idx and idx + 1 < len(longs) and longs[idx + 1][0][0] != 'g':
            o.append("p%d" % pend.pop(0)[0])
    assert t == 16 and not pend
    return o


def _order_first(n1, n2, n3):
    o = _seq("k", 0, n1) + ["K"] + _seq("s", 0, n1)
    o += _zip(_seq("k", n1, n2), _seq("p", 0, n1)) + ["Q"] + _seq("s", n1, n2)
    o += _zip(_seq("k", n2, n3), _seq("p", n1, n2)) + ["V"] + _seq("s", n2, n3)
    done = n2
    for t in range(n3, 32):
        o += ["q%d" % t] + (["s%d" % (t - 1)] if t > n3 else [])
        for _ in range(2 if done < 15 else 1):
            if done <= t - 2:
                o += ["p%d" % done] + (["F"] if done == 15 else [])
                done += 1
    return o + ["u31"] + _seq("p", done, 32)


ORDER_MID = _order_mid([3, 3, 2, 2, 2, 2, 2], 2)
ORDER_FIRST = _order_first(8, 11, 14)
ORDER_LAST = "f G0 g1 g2 g3 g4 g5 g6 d0 d1 d2 d3 D4".split()
CF, CM = (80, 180), (104, 180)
PM, PM6, PMQ = (0, 1, 1, 2), (0, 0, 1, 1), (0, 1, 2, 3)


def make_kernel():
    def kernel(x_hbm, wqkv_hbm, wo_hbm, wg_hbm, wu_hbm, wd_hbm, o_hbm,
               x_s, wqkv_s, wo_s, wgu_s, wd_s, sems, kbuf, vbuf, qt, qt0, at_ref, at0_ref,
               attn_s, s_ref, p_ref, o_s):
        step = pl.program_id(0)
        zero_rt = step >> 8

        def rows(b, n):
            if isinstance(b, int):
                return pl.ds(b * n, n)
            return pl.ds(pl.multiple_of(b * n, n), n)

        class Ring:
            def __init__(self, ref, n, cap):
                assert cap * n <= ref.shape[0]
                self.ref, self.n, self.cap, self.ptr, self.live = ref, n, cap, 0, set()
                self.always = _iota((n, 128), 1) >= zero_rt

            def put(self, val):
                k = self.ptr
                self.ptr = (k + 1) % self.cap
                assert k not in self.live
                self.live.add(k)
                pltpu.store(self.ref.at[pl.ds(k * self.n, self.n), :], val, mask=self.always)
                return k

            def get(self, k):
                self.live.remove(k)
                return self.ref[k * self.n:(k + 1) * self.n, :]

        def xcp(b):
            sl = pl.ds(b * T, T if b < 3 else S - b * T)
            return pltpu.make_async_copy(x_hbm.at[sl], x_s.at[sl], sems.at[(5, 3, 4, 5)[b]])

        def ocp(b, c):
            return pltpu.make_async_copy(o_s.at[rows(b & 1, T), 128 * c:128 * (c + 1)],
                                         o_hbm.at[rows(b, T), 128 * c:128 * (c + 1)], sems.at[7])

        def ocp_full(b):
            return pltpu.make_async_copy(o_s.at[rows(b & 1, T)], o_hbm.at[rows(b, T)], sems.at[6])

        def cp(name):
            mk = pltpu.make_async_copy
            if name[0] == 'c':
                n = int(name[1])
                return [mk(wqkv_hbm.at[:, QC[n]:QC[n + 1]], wqkv_s.at[:, QC[n]:QC[n + 1]], sems.at[n])]
            if name[0] == 'x':
                return [xcp(int(name[1]))]
            if name == 'wo':
                return [mk(wo_hbm, wo_s, sems.at[4])]
            if name == 'gu':
                return [mk(wg_hbm.at[0:FM], wgu_s.at[0:FM], sems.at[4]),
                        mk(wu_hbm.at[0:FM], wgu_s.at[FM:2 * FM], sems.at[4]),
                        mk(wg_hbm.at[FM:F], wgu_s.at[2 * FM:2 * FM + 64], sems.at[4]),
                        mk(wu_hbm.at[FM:F], wgu_s.at[2 * FM + 64:2 * F], sems.at[4])]
            return [mk(wd_hbm, wd_s, sems.at[4])]

        def wait(*names):
            for n in names:
                for c in cp(n):
                    c.wait()

        def ln1(b):
            return _ln(x_s[rows(b, T), :].astype(f32)).astype(bf16)

        def proj(ln, c0, c1):
            return jnp.dot(ln, wqkv_s[:, c0:c1], preferred_element_type=f32)

        def put_q(q, dst):
            q = q * (DH ** -0.5 * LOG2E)
            hh = (_iota((1, D), 1) * 3277) >> 16
            h0, h1 = (hh & 1) == 1, (hh & 2) == 2
            out = []
            for qb in range(NQ):
                a = [q[qb * 128 + 32 * c:qb * 128 + 32 * c + 32] for c in range(4)]
                b = [jnp.where(h0, a[(c - 1) % 4], a[c]) for c in range(4)]
                out += [jnp.where(h1, b[(c - 2) % 4], b[c]) for c in range(4)]
            dst[...] = _pk(jnp.concatenate(out, axis=0).T)

        def put_k(k, roll, first=False):
            o = 0 if first else W2
            lane = _iota((1, 128), 1)
            for i in range(8):
                gh, gl = _win_src(i)
                w = k[:, gh * 128:(gh + 1) * 128]
                if gl != gh:
                    w = jnp.where(lane >= 64, w, k[:, gl * 128:(gl + 1) * 128])
                if roll:
                    kbuf[i * KR:i * KR + W2, :] = kbuf[i * KR + T2:(i + 1) * KR, :]
                kbuf[i * KR + o:i * KR + o + T2, :] = _pk(w)

        def put_v(v, roll, first=False):
            o = 0 if first else W
            vt = v.T
            row = _iota((24, 1), 0)
            if roll:
                vbuf[:, 0:W] = vbuf[:, T:T + W]
            for h in range(H):
                base = 8 * ((20 * h) // 8)
                vbuf[24 * h:24 * h + 24, o:o + T] = jnp.where(row == _ones_row(h), 1.0,
                                                              vt[base:base + 24, :])

        class Attn:
            def __init__(self, units, caps):
                self.tri = _iota((32, 128), 0) > (_iota((32, 128), 1) & 31)
                self.never = _iota((8, 128), 1) < zero_rt
                lane = _iota((16, 128), 1)
                self.b0, self.b1 = (lane & 32) == 0, (lane & 64) == 0
                self.z8, self.z16, self.z40 = (jnp.zeros((n, 128), u32) for n in (8, 16, 40))
                self.zf, self.neg = jnp.zeros((32, 128), f32), jnp.full((32, 128), NEG, f32)
                code = ((_iota((40, 128), 1) >> 5) - ((_iota((40, 128), 0) * 6554) >> 16)) & 3
                self.qsel = [code == j for j in range(4)]
                self.units, self.st, self.pt = units, {}, {}
                self.sr, self.pr = Ring(s_ref, 32, caps[0]), Ring(p_ref, 16, caps[1])

            def qk(self, t):
                first, i, qb = self.units[t]
                res, pace = [], []
                for j in range(4):
                    k0 = i * KR + qb * 64 + 16 * j - (W2 if first else 0)
                    rm = max(0, 8 - (qb * 4 + j)) if first else 0
                    lo = max(rm, 1)
                    parts = [kbuf[k0:k0 + 16, :]] if rm == 0 else []
                    parts.append(kbuf[k0 + 128:k0 + 144, :])
                    if lo < 8:
                        parts.append(kbuf[k0 + 16 * lo:k0 + 128, :])
                    lhs = jnp.concatenate(parts, axis=0) if len(parts) > 1 else parts[0]
                    qs = (qt0 if first else qt)[40 * i:40 * i + 40, qb * 128:(qb + 1) * 128]
                    qs = lax.select(self.qsel[j], qs, self.z40)
                    pos = [self.z8] * 8
                    for v in range(5):
                        pos[(5 * i + v) % 8] = qs[8 * v:8 * v + 8]
                    sp = jnp.dot(_up(lhs), _up(jnp.concatenate(pos, axis=0)),
                                 preferred_element_type=f32)
                    o = 64 if rm == 0 else 32
                    edge = lax.select(self.tri, sp[0:32] if rm == 0 else self.neg, sp[o - 32:o])
                    chunks = [(0, edge)] + [(r, sp[o + 32 * (r - lo):o + 32 * (r - lo + 1)])
                                            for r in range(lo, 8)]
                    run = []
                    for _, c in chunks:
                        cm = jnp.maximum(jnp.maximum(c[0:8], c[8:16]), jnp.maximum(c[16:24], c[24:32]))
                        run.append(jnp.maximum(run[-1], cm) if run else cm)
                    m8 = jnp.broadcast_to(jnp.max(run[-1], axis=0, keepdims=True), (8, 128))
                    res.append(([(r, self.sr.put(c)) for r, c in chunks], m8, rm))
                    pace.append(run)
                self.st[t] = res
                return pace

            def sm(self, t, pace):
                cur = self.st.pop(t)
                P = [[None] * 9 for _ in range(4)]
                for n in range(8):
                    for j in range(4):
                        chunks, m, rm = cur[j]
                        if n >= len(chunks):
                            continue
                        r, s = chunks[n]
                        if pace is not None:
                            m = lax.select(self.never, pace[j][min(n, len(pace[j]) - 1)], m)
                        p = jnp.exp2(self.sr.get(s).reshape(4, 8, 128) - m[None]).reshape(32, 128)
                        if r > 0:
                            P[j][r] = _pk(p)
                        elif rm == 0:
                            P[j][0] = _pk(lax.select(self.tri, p, self.zf))
                            P[j][8] = _pk(lax.select(self.tri, self.zf, p))
                        else:
                            P[j][8] = _pk(p)
                self.pt[t] = [[None if z is None else self.pr.put(z) for z in P[j]] for j in range(4)]

            def sel(self, m, a, b):
                if a is None and b is None:
                    return None
                return lax.select(m, self.z16 if a is None else a, self.z16 if b is None else b)

            def pv(self, t):
                first, i, qb = self.units[t]
                P = self.pt.pop(t)
                acc = [None] * 4
                for kt in range(max(0, 2 - qb) if first else 0, 3):
                    B = [[None] * 4 for _ in range(4)]
                    for r4 in range(4):
                        r = 4 * kt + r4
                        A = [P[j][r - j] if 0 <= r - j <= 8 else None for j in range(4)]
                        A = [None if a is None else self.pr.get(a) for a in A]
                        C = [self.sel(self.b0, A[j], A[(j + 1) % 4]) for j in range(4)]
                        for j in range(4):
                            b = self.sel(self.b1, C[j], C[(j + 2) % 4])
                            B[(-j) % 4][r4] = self.z16 if b is None else b
                    c0 = qb * 128 + kt * 128 - (W if first else 0)
                    for hh in range(4):
                        h = 4 * i + hh
                        d = jnp.dot(vbuf[24 * h:24 * h + 24, c0:c0 + 128],
                                    _up(jnp.concatenate(B[hh], axis=0)),
                                    precision=lax.Precision.DEFAULT, preferred_element_type=f32)
                        acc[hh] = d if acc[hh] is None else acc[hh] + d
                dst = at0_ref if first else at_ref
                for hh in range(4):
                    off, one = (20 * hh) % 8, _ones_row(hh)
                    o = acc[hh] * (1.0 / acc[hh][one:one + 1, :])
                    if hh:
                        o = pltpu.roll(o, 128 - 32 * hh, 1)
                    dst[i, 20 * hh:20 * hh + 20, qb * 128:(qb + 1) * 128] = o[off:off + 20, :]

        def fin(src, slot):
            attn_s[rows(slot, T2), :] = _pk(src[...].reshape(D, T).T)

        def pace_of(z, tiles):
            return [[z[32 * m:32 * m + 8, 128 * c:128 * c + 128] for m in range(8)] for c in tiles]

        class Ffn:
            def __init__(self, b, tail):
                split = 2 if tail else 1
                R = T // split
                at = _up(attn_s[rows(b & 1, T2), :])
                x = x_s[rows(b, T), :].astype(f32)
                h1 = [x[s * R:(s + 1) * R] + jnp.dot(at[s * R:(s + 1) * R], wo_s[...],
                                                     preferred_element_type=f32)
                      for s in range(split)]
                self.ln2 = [_ln(h, 0.5).astype(bf16) for h in h1]
                self.h1 = jnp.concatenate(h1, axis=0) if tail else h1[0]
                self.hs, self.b, self.tail = {}, b, tail

            def gu(self, c, split):
                n = 256 if c < 6 else 128
                w = jnp.concatenate([wgu_s[256 * c:256 * c + n, :],
                                     wgu_s[FM + 256 * c:FM + 256 * c + 256, :]], axis=0)
                ls = self.ln2 if split or not self.tail else [jnp.concatenate(self.ln2, axis=0)]
                gu = [lax.dot_general(l, w, NT, preferred_element_type=f32) for l in ls]
                gu = jnp.concatenate(gu, axis=0) if len(gu) > 1 else gu[0]
                self.hs[c] = _glu(gu[:, 0:n], gu[:, n:2 * n])
                if c == 6:
                    self.hs[7] = _glu(gu[:, 256:320], gu[:, 320:384])
                if len(self.hs) == 8:
                    self.hh = jnp.concatenate([self.hs[u] for u in range(8)], axis=1).astype(bf16)
                return None if self.tail else pace_of(gu, PM if c < 6 else PM6)

            def down(self, c, split):
                R = T // split
                for s in range(split):
                    y = jnp.dot(self.hh[s * R:(s + 1) * R], wd_s[:, 128 * c:128 * (c + 1)],
                                preferred_element_type=f32)
                    o_s[rows((self.b & 1) * split + s, R), 128 * c:128 * (c + 1)] = (
                        self.h1[s * R:(s + 1) * R, 128 * c:128 * (c + 1)] + y).astype(bf16)
                if self.tail:
                    ocp(self.b, c).start()

        def run(order, at, ff, ln, roll):
            pace = None
            for tok in order:
                k, n = tok[0], (int(tok[1:]) if tok[1:] else None)
                if k == 'k':
                    at.qk(n)
                elif k == 'q':
                    pace = at.qk(n)
                elif k in 'su':
                    at.sm(n, pace if k == 's' else None)
                elif k == 'p':
                    at.pv(n)
                elif k in 'gG':
                    pace = ff.gu(n, k == 'G')
                elif k in 'dD':
                    ff.down(n, 2 if k == 'D' else 1)
                elif k == 'f':
                    fin(at_ref, step & 1)
                elif k == 'F':
                    fin(at0_ref, 0)
                else:
                    c0 = 'QKV'.index(k) * D
                    z = proj(ln, c0, c0 + D)
                    pace = None if roll else pace_of(z, PMQ)
                    if k == 'Q':
                        put_q(z, qt)
                    elif k == 'K':
                        put_k(z, roll)
                    else:
                        put_v(z, roll)

        std = [(False, i, qb) for qb in range(NQ) for i in range(8)]

        def first():
            for n in ['x0', 'c0', 'c1', 'c2', 'x1', 'c3', 'wo', 'x2', 'gu', 'wd']:
                for c in cp(n):
                    c.start()
            s_ref[...] = jnp.zeros(s_ref.shape, f32)
            p_ref[...] = jnp.zeros(p_ref.shape, u32)
            wait('x0')
            ln = ln1(0)
            zs = []
            for c in range(4):
                wait('c%d' % c)
                if c == 3:
                    wait('x1')
                zs.append(proj(ln, QC[c], QC[c + 1]))
            z = jnp.concatenate(zs, axis=1)
            ln = ln1(1)
            put_k(z[:, D:2 * D], False, True)
            put_q(z[:, 0:D], qt0)
            put_v(z[:, 2 * D:3 * D], False, True)
            units = [(True, i, qb) for qb in range(NQ) for i in range(8)] + std
            run(ORDER_FIRST, Attn(units, CF), None, ln, False)
            wait('wo', 'x2', 'gu', 'wd')
            xcp(3).start()

        def middle():
            @pl.when(step >= 2)
            def _():
                ocp_full(step - 2).start()
            ff = Ffn(step - 1, False)
            run(ORDER_MID, Attn(std, CM), ff, ln1(step + 1), True)

            @pl.when(step >= 2)
            def _():
                ocp_full(step - 2).wait()

            @pl.when(step == 1)
            def _():
                xcp(3).wait()

        def last():
            @pl.when(step == NB - 1)
            def _():
                ocp_full(NB - 3).start()
            run(ORDER_LAST, None, Ffn(step - 1, True), None, None)

            @pl.when(step == NB - 1)
            def _():
                ocp_full(NB - 3).wait()

            @pl.when(step == NB)
            def _():
                for b in (NB - 2, NB - 1):
                    for c in range(5):
                        ocp(b, c).wait()

        lax.cond(jnp.logical_and(step > 0, step < NB - 1), middle,
                 lambda: lax.cond(step == 0, first, last))

    return kernel


@jax.jit
def pallas_sequential_preLN__sliding_block__glu_gated_glu__prompt_kernel(
    A_x: jax.Array,
    A_wqkv: jax.Array,
    A_wo: jax.Array,
    B_x: jax.Array,
    B_w_gate: jax.Array,
    B_w_up: jax.Array,
    B_w_down: jax.Array,
):
    del B_x
    hbm = pl.BlockSpec(memory_space=pl.ANY)
    out = pl.pallas_call(
        make_kernel(),
        grid=(NB + 1,),
        in_specs=[hbm] * 6,
        out_specs=hbm,
        out_shape=jax.ShapeDtypeStruct((S, D), bf16),
        scratch_shapes=[pltpu.VMEM((S, D), bf16),
                        pltpu.VMEM((D, 3 * D), bf16),
                        pltpu.VMEM((D, D), bf16),
                        pltpu.VMEM((2 * F, D), bf16),
                        pltpu.VMEM((F, D), bf16),
                        pltpu.SemaphoreType.DMA((8,)),
                        pltpu.VMEM((8 * KR, 128), u32),
                        pltpu.VMEM((H * 24, W + T), f32),
                        pltpu.VMEM((D // 2, T), u32),
                        pltpu.VMEM((D // 2, T), u32),
                        pltpu.VMEM((8, 80, T), f32),
                        pltpu.VMEM((8, 80, T), f32),
                        pltpu.VMEM((2 * T2, D), u32),
                        pltpu.VMEM((max(CF[0], CM[0]) * 32, 128), f32),
                        pltpu.VMEM((max(CF[1], CM[1]) * 16, 128), u32),
                        pltpu.VMEM((2 * T, D), bf16)],
        compiler_params=pltpu.CompilerParams(dimension_semantics=("arbitrary",),
                                             vmem_limit_bytes=64 * 1024 * 1024),
    )(A_x.reshape(S, D), A_wqkv, A_wo, B_w_gate.T, B_w_up.T, B_w_down)
    return out.reshape(1, S, D)
```
